```python
import os as _os
_os.environ.setdefault('JAX_PLATFORMS', 'cpu')
import jax
import jax.numpy as jnp

def _softmax(x, axis=-1):
    return jax.nn.softmax(x, axis=axis)

def _gelu(x):
    return jax.nn.gelu(x, approximate=True)

def _silu(x):
    return jax.nn.silu(x)

def _sigmoid(x):
    return jax.nn.sigmoid(x)

def _layernorm(x, axis=-1, eps=1e-05):
    m = jnp.mean(x, axis=axis, keepdims=True)
    v = jnp.var(x, axis=axis, keepdims=True)
    return (x - m) / jnp.sqrt(v + eps)

def _scatter_add(tgt, idx, src, axis=0):
    return tgt.at[idx].add(src)

def _segment_sum(src, seg, n):
    return jax.ops.segment_sum(src, seg, n)

class _Rng:

    def __init__(self, key):
        self._k = key

    def _next(self):
        self._k, sub = jax.random.split(self._k)
        return sub

    def normal(self, shape):
        return jax.random.normal(self._next(), shape, dtype=jnp.bfloat16)

    def randint(self, lo, hi, shape):
        return jax.random.randint(self._next(), shape, lo, hi, dtype=jnp.int32)

    def uniform(self, shape, lo=0.0, hi=1.0):
        return jax.random.uniform(self._next(), shape, jnp.bfloat16, lo, hi)

    def permutation(self, n):
        return jax.random.permutation(self._next(), n)
kernel_name = 'sequential_preLN__memory_aug_recurrent_mem_tr__swiglu_ffn__prompt'

def setup_inputs():
    _rng = _Rng(jax.random.key(int.from_bytes(__import__("os").urandom(4), "little")))
    _w = lambda a: (lambda t: t.astype(jnp.bfloat16) if jnp.issubdtype(t.dtype, jnp.floating) else t)(jnp.asarray(a))

    def _A_setup():
        B, S, Dm = (1, 2048, 640)
        H, Dh = (32, 192)
        M, seg = (8, 32)
        seg = min(seg, S)
        S = S // seg * seg
        return {'x': _w((lambda *s: _rng.normal(s) * 0.05)(B, S, Dm)), 'mem0': _w((lambda *s: _rng.normal(s) * 0.1)(B, M, Dm)), 'Wq': _w((lambda *s: _rng.normal(s) * 1.6)(Dm, H, Dh) * Dm ** (-0.5)), 'Wk': _w((lambda *s: _rng.normal(s) * 1.6)(Dm, H, Dh) * Dm ** (-0.5)), 'Wv': _w((lambda *s: _rng.normal(s) * 0.1)(Dm, H, Dh) * Dm ** (-0.5)), 'Wo': _w((lambda *s: _rng.normal(s) * 0.1)(H, Dh, Dm) * (H * Dh) ** (-0.5)), 'seg_len': seg}
    _A_in = _A_setup()

    def _B_setup():
        B, S, D, F = (1, 2048, 640, 1536)
        return {'x': _w((lambda *s: _rng.normal(s) * 0.05)(B, S, D)), 'w_gate': _w((lambda *s: _rng.normal(s) * 0.05)(D, F)), 'w_up': _w((lambda *s: _rng.normal(s) * 0.05)(D, F)), 'w_down': _w((lambda *s: _rng.normal(s) * 0.05)(F, D))}
    _B_in = _B_setup()
    return {'A_x': _A_in['x'], 'A_mem0': _A_in['mem0'], 'A_Wq': _A_in['Wq'], 'A_Wk': _A_in['Wk'], 'A_Wv': _A_in['Wv'], 'A_Wo': _A_in['Wo'], 'A_seg_len': _A_in['seg_len'], 'B_x': _B_in['x'], 'B_w_gate': _B_in['w_gate'], 'B_w_up': _B_in['w_up'], 'B_w_down': _B_in['w_down']}

def reference(A_x, A_mem0, A_Wq, A_Wk, A_Wv, A_Wo, A_seg_len, B_x, B_w_gate, B_w_up, B_w_down):

    def _A_ref(x, mem0, Wq, Wk, Wv, Wo, seg_len):
        B, S, Dm = x.shape
        H, Dh = (Wq.shape[1], Wq.shape[2])
        M = mem0.shape[1]
        scale = Dh ** (-0.5)
        n_seg = S // seg_len
        L = M + seg_len
        idx = jnp.arange(L)
        mask = (idx[:, None] < M) | (idx[:, None] >= idx[None, :])
        mem = mem0
        outs = []
        for s in range(n_seg):
            xs = x[:, s * seg_len:(s + 1) * seg_len, :].copy()
            h = jnp.concatenate([mem, xs], axis=1)
            q = jnp.einsum('btd,dhe->bhte', h, Wq)
            k = jnp.einsum('btd,dhe->bhte', h, Wk)
            v = jnp.einsum('btd,dhe->bhte', h, Wv)
            scores = jnp.einsum('bhqe,bhke->bhqk', q, k) * scale
            scores = jnp.where(mask[None, None], scores, -1000000000.0)
            p = _softmax(scores, axis=-1)
            o = jnp.einsum('bhqk,bhke->bhqe', p, v)
            o = jnp.einsum('bhte,hed->btd', o, Wo)
            mem = o[:, :M, :].copy()
            outs.append(o[:, M:, :])
        return jnp.concatenate(outs, axis=1)

    def _B_ref(x, w_gate, w_up, w_down):
        g = _silu(x @ w_gate)
        u = x @ w_up
        return g * u @ w_down
    x = A_x
    h = x + _A_ref(_layernorm(x, axis=-1), A_mem0, A_Wq, A_Wk, A_Wv, A_Wo, A_seg_len)
    h2 = h + _B_ref(_layernorm(h, axis=-1), B_w_gate, B_w_up, B_w_down)
    return h2
```

```python
import functools

import jax
import jax.numpy as jnp
import jax.experimental.pallas as pl
import jax.experimental.pallas.tpu as pltpu

_F32 = jnp.float32
_BF16 = jnp.bfloat16
_U32 = jnp.uint32
_NN = (((1,), (0,)), ((), ()))
_NT = (((1,), (1,)), ((), ()))


def _mm(a, b, dims=_NN):
    return jax.lax.dot_general(a, b, dims, preferred_element_type=_F32)


def _layernorm(x):
    m = jnp.mean(x, axis=-1, keepdims=True)
    d = x - m
    v = jnp.mean(d * d, axis=-1, keepdims=True)
    return d / jnp.sqrt(v + 1e-5)


def _kernel(x_hbm, mem0_ref, wq_hbm, wk_hbm, wv_hbm, wo_hbm, wg_hbm, wu_hbm, wd_hbm, out_hbm,
            xbuf, xn, stq, stk, stv, wqkv, wo, wg, wu, wd, obuf, sem_w, sem_m, sem_o,
            *, S, D, H, Dh, M, seg):
    n_seg = S // seg
    n_pair = H // 2
    PW = 2 * Dh
    L = M + seg
    scale = Dh ** -0.5

    def w_copies(p):
        rows = pl.ds(p * PW, PW)
        return [pltpu.make_async_copy(src.at[rows], dst.at[p], sem_w.at[i, p])
                for i, (src, dst) in enumerate(((wq_hbm, stq), (wk_hbm, stk), (wv_hbm, stv)))]

    x_copy = pltpu.make_async_copy(x_hbm, xbuf, sem_m.at[0])
    rest = [pltpu.make_async_copy(src, dst.bitcast(_BF16), sem_m.at[i + 1])
            for i, (src, dst) in enumerate(((wo_hbm, wo), (wg_hbm, wg), (wu_hbm, wu), (wd_hbm, wd)))]
    x_copy.start()
    for p in range(n_pair):
        for c in w_copies(p):
            c.start()
    for c in rest:
        c.start()

    x_copy.wait()

    def ln_body(s, _):
        rows = pl.ds(pl.multiple_of(s * 64, 64), 64)
        xn[rows, :] = _layernorm(xbuf[rows, :].astype(_F32))
        return 0
    jax.lax.fori_loop(0, S // 64, ln_body, 0)

    def w_body(p, _):
        for c in w_copies(p):
            c.wait()
        for i, st in enumerate((stq, stk, stv)):
            wqkv[p, :, i * PW:(i + 1) * PW] = pltpu.bitcast(st[p].T, _U32)
        return 0
    jax.lax.fori_loop(0, n_pair, w_body, 0)
    for c in rest:
        c.wait()

    def block_diag(t):
        lane = jax.lax.broadcasted_iota(jnp.int32, t.shape, 1)
        is_a = lane < Dh
        return jnp.concatenate([jnp.where(is_a, t, 0.0), jnp.where(is_a, 0.0, t)], axis=0).astype(_BF16)

    def step(s, mem):
        rows = pl.ds(pl.multiple_of(s * seg, seg), seg)
        h = jnp.concatenate([mem, xn[rows, :]], axis=0)

        row = jax.lax.broadcasted_iota(jnp.int32, (L, 2 * L), 0)
        col = jax.lax.broadcasted_iota(jnp.int32, (L, 2 * L), 1)
        head_a = col < L
        key = jnp.where(head_a, col, col - L)
        allowed = (row < M) | (row >= key)

        def proj(p):
            return _mm(h, pltpu.bitcast(wqkv[p], _BF16))

        acc = None
        qkv = proj(0)
        for p in range(n_pair):
            q, k, v = qkv[:, :PW], qkv[:, PW:2 * PW], qkv[:, 2 * PW:]
            sc = _mm(q, block_diag(k), _NT) * scale
            if p + 1 < n_pair:
                qkv = proj(p + 1)
            sc = jnp.where(allowed, sc, -1e9)
            m_a = jnp.max(jnp.where(head_a, sc, -jnp.inf), axis=-1, keepdims=True)
            m_b = jnp.max(jnp.where(head_a, -jnp.inf, sc), axis=-1, keepdims=True)
            e = jnp.exp(sc - jnp.where(head_a, m_a, m_b))
            l_a = jnp.sum(jnp.where(head_a, e, 0.0), axis=-1, keepdims=True)
            l_b = jnp.sum(jnp.where(head_a, 0.0, e), axis=-1, keepdims=True)
            prob = e / jnp.where(head_a, l_a, l_b)
            o = _mm(prob, block_diag(v))
            c = _mm(o, pltpu.bitcast(wo[p * Dh:(p + 1) * Dh, :], _BF16))
            acc = c if acc is None else acc + c

        hres = xbuf[rows, :].astype(_F32) + acc[M:]
        hn = _layernorm(hres)
        g = _mm(hn, pltpu.bitcast(wg[...], _BF16))
        u = _mm(hn, pltpu.bitcast(wu[...], _BF16))
        a = g * jax.nn.sigmoid(g) * u
        y = hres + _mm(a, pltpu.bitcast(wd[...], _BF16))
        obuf[rows, :] = y.astype(_BF16)
        pltpu.make_async_copy(obuf.at[rows], out_hbm.at[rows], sem_o).start()
        return acc[:M]

    jax.lax.fori_loop(0, n_seg, step, mem0_ref[...].astype(_F32))
    pltpu.make_async_copy(obuf, out_hbm, sem_o).wait()


@functools.partial(jax.jit, static_argnames=("A_seg_len",))
def pallas_sequential_preLN__memory_aug_recurrent_mem_tr__swiglu_ffn__prompt_kernel(
    A_x: jax.Array,
    A_mem0: jax.Array,
    A_Wq: jax.Array,
    A_Wk: jax.Array,
    A_Wv: jax.Array,
    A_Wo: jax.Array,
    A_seg_len: int,
    B_x: jax.Array,
    B_w_gate: jax.Array,
    B_w_up: jax.Array,
    B_w_down: jax.Array,
):
    del B_x
    B, S, D = A_x.shape
    _, H, Dh = A_Wq.shape
    M = A_mem0.shape[1]
    F = B_w_gate.shape[1]
    seg = int(A_seg_len)
    assert B == 1 and S % seg == 0 and H % 2 == 0
    n_pair = H // 2

    def t(w):
        return jnp.transpose(w, (1, 2, 0)).reshape(H * Dh, D)

    hbm = pl.BlockSpec(memory_space=pl.ANY)
    out = pl.pallas_call(
        functools.partial(_kernel, S=S, D=D, H=H, Dh=Dh, M=M, seg=seg),
        out_shape=jax.ShapeDtypeStruct((S, D), A_x.dtype),
        in_specs=[hbm, pl.BlockSpec(memory_space=pltpu.VMEM)] + [hbm] * 7,
        out_specs=hbm,
        scratch_shapes=[
            pltpu.VMEM((S, D), _BF16),
            pltpu.VMEM((S, D), _F32),
            pltpu.VMEM((n_pair, 2 * Dh, D), _BF16),
            pltpu.VMEM((n_pair, 2 * Dh, D), _BF16),
            pltpu.VMEM((n_pair, 2 * Dh, D), _BF16),
            pltpu.VMEM((n_pair, D // 2, 6 * Dh), _U32),
            pltpu.VMEM((H * Dh // 2, D), _U32),
            pltpu.VMEM((D // 2, F), _U32),
            pltpu.VMEM((D // 2, F), _U32),
            pltpu.VMEM((F // 2, D), _U32),
            pltpu.VMEM((S, D), _BF16),
            pltpu.SemaphoreType.DMA((3, n_pair)),
            pltpu.SemaphoreType.DMA((5,)),
            pltpu.SemaphoreType.DMA(()),
        ],
        compiler_params=pltpu.CompilerParams(vmem_limit_bytes=110 * 2**20),
    )(A_x.reshape(S, D), A_mem0.reshape(M, D), t(A_Wq), t(A_Wk), t(A_Wv), A_Wo.reshape(H * Dh, D),
      B_w_gate, B_w_up, B_w_down)
    return out.reshape(B, S, D)
```

```python
import functools
import math

import jax
import jax.numpy as jnp
import jax.experimental.pallas as pl
import jax.experimental.pallas.tpu as pltpu

_F32 = jnp.float32
_BF16 = jnp.bfloat16
_U32 = jnp.uint32
_NN = (((1,), (0,)), ((), ()))
_NT = (((1,), (1,)), ((), ()))
_LANES = 128
_SIDE_SLOTS = 3


def _mm(a, b, dims=_NN):
    return jax.lax.dot_general(a, b, dims, preferred_element_type=_F32)


def _layernorm(x):
    m = jnp.mean(x, axis=-1, keepdims=True)
    d = x - m
    v = jnp.mean(d * d, axis=-1, keepdims=True)
    return d / jnp.sqrt(v + 1e-5)


def _aligned(i, n):
    return i if isinstance(i, int) else pl.multiple_of(i, n)


def _pack(w):
    return pltpu.bitcast(w, _U32)


def _unpack(w):
    return pltpu.bitcast(w, _BF16)


def _kernel(x_hbm, mem0_hbm, wq_hbm, wk_hbm, wv_hbm, wo_hbm, wg_hbm, wu_hbm, wd_hbm, out_hbm,
            xbuf, xn0, stage, wqkv, wo, wg, wu, wd, ring0, ring1, obuf, hres, xn1, mem0,
            so, sg, su, sd, sem_w, sem_s, sem_m, sem_o, *, H, Dh, seg):
    S, D = xbuf.shape
    M = mem0_hbm.shape[0]
    F = wu_hbm.shape[1]
    n_seg = S // seg
    n_pair = H // 2
    PW = 2 * Dh
    L = M + seg
    scale = Dh ** -0.5
    adv = seg - M
    ahead = M * n_seg
    rings = (ring0, ring1)
    R = ring0.shape[1]
    off = R - ahead

    def pair_copies(p):
        rows = pl.ds(_aligned(p * PW, PW), PW)
        return [pltpu.make_async_copy(src.at[rows], stage.at[p, pl.ds(i * PW, PW)], sem_w.at[i, p])
                for i, src in enumerate((wk_hbm, wq_hbm, wv_hbm))]

    n_side = n_pair // 2 - 2
    side = ((wo_hbm, so, wo), (wg_hbm, sg, wg), (wu_hbm, su, wu), (wd_hbm, sd, wd))

    def side_start(j, src, st):
        n = st.shape[1]
        return jnp.minimum(j * n, src.shape[0] - n)

    def side_copies(j):
        slot = j % _SIDE_SLOTS
        return [pltpu.make_async_copy(src.at[pl.ds(_aligned(side_start(j, src, st), 16), st.shape[1])],
                                      st.at[slot], sem_s.at[i, slot])
                for i, (src, st, _) in enumerate(side)]

    def side_pack(j):
        for src, st, dst in side:
            rows = pl.ds(_aligned(side_start(j, src, st) // 2, 8), st.shape[1] // 2)
            dst[rows, :] = _pack(st[j % _SIDE_SLOTS])

    def lead_pair(g, r):
        p = 2 * g + r
        for i in range(3):
            cols = slice(i * PW, (i + 1) * PW)
            w = stage[p, cols, :]
            rings[r][g, off:, cols] = _mm(xn0[...], w, _NT)
            wqkv[p, :, cols] = _pack(w.T)

    x_head = pltpu.make_async_copy(x_hbm.at[:ahead], xbuf.at[:ahead], sem_m.at[0])
    x_tail = pltpu.make_async_copy(x_hbm.at[ahead:], xbuf.at[ahead:], sem_m.at[1])
    mem_copy = pltpu.make_async_copy(mem0_hbm, mem0.at[0], sem_m.at[2])
    x_head.start()
    mem_copy.start()
    for c in pair_copies(0):
        c.start()
    x_head.wait()
    xn0[...] = _layernorm(xbuf[:ahead, :].astype(_F32)).astype(_BF16)
    for c in pair_copies(1):
        c.start()

    def lead_body(p, _):
        g = p // 2
        for c in pair_copies(p):
            c.wait()

        @pl.when(p + 2 < n_pair)
        def _():
            for c in pair_copies(p + 2):
                c.start()

        @pl.when(p % 2 == 0)
        def _():
            @pl.when(g >= 2)
            def _():
                for c in side_copies(g - 2):
                    c.wait()
                side_pack(g - 2)
            lead_pair(g, 0)

        @pl.when(p % 2 == 1)
        def _():
            @pl.when(g < n_side)
            def _():
                for c in side_copies(g):
                    c.start()

            @pl.when(g == n_side)
            def _():
                x_tail.start()
            lead_pair(g, 1)
        return 0

    jax.lax.fori_loop(0, n_pair, lead_body, 0)
    x_tail.wait()
    mem_copy.wait()

    def block_diag(t):
        is_a = jax.lax.broadcasted_iota(jnp.int32, t.shape, 1) < Dh
        pad = jnp.zeros((_LANES - 2 * L, PW), _F32)
        return jnp.concatenate([jnp.where(is_a, t, 0.0), jnp.where(is_a, 0.0, t), pad], axis=0).astype(_BF16)

    def rows_of(s):
        return pl.ds(_aligned(s * seg, seg), seg)

    def out_copy(s):
        return pltpu.make_async_copy(obuf.at[rows_of(s)], out_hbm.at[rows_of(s)], sem_o)

    def ffn_gate(hn):
        g = _mm(hn, _unpack(wg[...]))
        return g * jax.nn.sigmoid(g)

    def ffn_up(hn, cols=slice(None)):
        return _mm(hn, _unpack(wu[:, cols]))

    def ffn_down(s, a):
        y = hres[...] + _mm(a.astype(_BF16), _unpack(wd[...]))
        obuf[rows_of(s), :] = y.astype(obuf.dtype)

    def ln_new(s):
        return _layernorm(xbuf[pl.ds(_aligned(ahead + s * adv, M), adv), :].astype(_F32))

    def step(s, mem):
        h = jnp.concatenate([mem, xn1[...]], axis=0).astype(_BF16)
        xn1[...] = ln_new(jnp.minimum(s + 1, n_seg - 1))
        put = pl.ds(pl.multiple_of(jax.lax.rem(s * adv, R), M), adv)
        get = pl.ds(pl.multiple_of(jax.lax.rem(s * seg + off, R), seg), seg)
        hn = _layernorm(hres[...]).astype(_BF16)

        row = jax.lax.broadcasted_iota(jnp.int32, (L, _LANES), 0)
        col = jax.lax.broadcasted_iota(jnp.int32, (L, _LANES), 1)
        head_a = col < L
        head_b = (col >= L) & (col < 2 * L)
        key = jnp.where(head_a, col, col - L)
        allowed = ((row < M) | (row >= key)) & (col < 2 * L)
        fill = jnp.where(col < 2 * L, -1e9, -jnp.inf)

        def proj(p):
            kqv = _mm(h, _unpack(wqkv[p]))
            ring = rings[p % 2]
            ring[p // 2, put, :] = kqv[M:]
            kqv = jnp.concatenate([kqv[:M], ring[p // 2, get, :]], axis=0)
            return kqv[:, :PW], kqv[:, PW:2 * PW], kqv[:, 2 * PW:]

        def probs(q, k):
            sc = _mm(q, block_diag(k), _NT) * scale
            sc = jnp.where(allowed, sc, fill)
            m_a = jnp.max(jnp.where(head_a, sc, -jnp.inf), axis=-1, keepdims=True)
            m_b = jnp.max(jnp.where(head_b, sc, -jnp.inf), axis=-1, keepdims=True)
            e = jnp.exp(sc - jnp.where(head_a, m_a, m_b))
            l_a = jnp.sum(jnp.where(head_a, e, 0.0), axis=-1, keepdims=True)
            l_b = jnp.sum(jnp.where(head_b, e, 0.0), axis=-1, keepdims=True)
            return e / jnp.where(head_a, l_a, l_b)

        kqv, v, prob, o = {}, {}, {}, {}
        acc = None
        half = F // 2
        for i in range(n_pair + 3):
            if i < n_pair:
                kqv[i] = proj(i)
            elif i == n_pair:
                g = ffn_gate(hn)
            elif i == n_pair + 1:
                a0 = g[:, :half] * ffn_up(hn, slice(0, half))
            else:
                a1 = g[:, half:] * ffn_up(hn, slice(half, F))
            if i >= 3:
                c = _mm(o.pop(i - 3), _unpack(wo[(i - 3) * Dh:(i - 2) * Dh, :]))
                acc = c if acc is None else acc + c
            if 1 <= i <= n_pair:
                k, q, v[i - 1] = kqv.pop(i - 1)
                prob[i - 1] = probs(q, k)
            if 2 <= i <= n_pair + 1:
                o[i - 2] = _mm(prob.pop(i - 2), block_diag(v.pop(i - 2)))
        ffn_down(jnp.maximum(s - 1, 0), jnp.concatenate([a0, a1], axis=1))
        hres[...] = xbuf[rows_of(s), :].astype(_F32) + acc[M:]

        @pl.when(s > 0)
        def _():
            out_copy(s - 1).start()
        return acc[:M]

    hres[...] = jnp.zeros(hres.shape, _F32)
    xn1[...] = ln_new(0)
    jax.lax.fori_loop(0, n_seg, step, mem0[0].astype(_F32), unroll=4)
    hn = _layernorm(hres[...]).astype(_BF16)
    ffn_down(n_seg - 1, ffn_gate(hn) * ffn_up(hn))
    out_copy(n_seg - 1).start()
    pltpu.make_async_copy(obuf, out_hbm, sem_o).wait()


@functools.partial(jax.jit, static_argnames=("A_seg_len",))
def pallas_sequential_preLN__memory_aug_recurrent_mem_tr__swiglu_ffn__prompt_kernel(
    A_x: jax.Array,
    A_mem0: jax.Array,
    A_Wq: jax.Array,
    A_Wk: jax.Array,
    A_Wv: jax.Array,
    A_Wo: jax.Array,
    A_seg_len: int,
    B_x: jax.Array,
    B_w_gate: jax.Array,
    B_w_up: jax.Array,
    B_w_down: jax.Array,
):
    del B_x
    B, S, D = A_x.shape
    _, H, Dh = A_Wq.shape
    M = A_mem0.shape[1]
    F = B_w_gate.shape[1]
    seg = int(A_seg_len)
    n_pair = H // 2
    adv, ahead = seg - M, M * (S // seg)
    period = math.lcm(adv, seg)
    ring_rows = period * pl.cdiv(ahead + adv, period)
    assert B == 1 and S % seg == 0 and H % 4 == 0 and n_pair > 4
    assert M % 8 == 0 and seg % 16 == 0 and ahead % seg == 0 and 2 * (M + seg) <= _LANES

    def t(w):
        return jnp.transpose(w, (1, 2, 0)).reshape(H * Dh, D)

    def chunk(rows, cols):
        return pltpu.VMEM((_SIDE_SLOTS, 16 * pl.cdiv(rows, 16 * (n_pair // 2 - 2)), cols), _BF16)

    hbm = pl.BlockSpec(memory_space=pl.ANY)
    out = pl.pallas_call(
        functools.partial(_kernel, H=H, Dh=Dh, seg=seg),
        out_shape=jax.ShapeDtypeStruct((S, D), A_x.dtype),
        in_specs=[hbm] * 9,
        out_specs=hbm,
        scratch_shapes=[
            pltpu.VMEM((S, D), _BF16),
            pltpu.VMEM((ahead, D), _BF16),
            pltpu.VMEM((n_pair, 6 * Dh, D), _BF16),
            pltpu.VMEM((n_pair, D // 2, 6 * Dh), _U32),
            pltpu.VMEM((H * Dh // 2, D), _U32),
            pltpu.VMEM((D // 2, F), _U32),
            pltpu.VMEM((D // 2, F), _U32),
            pltpu.VMEM((F // 2, D), _U32),
            pltpu.VMEM((n_pair // 2, ring_rows, 6 * Dh), _F32),
            pltpu.VMEM((n_pair // 2, ring_rows, 6 * Dh), _F32),
            pltpu.VMEM((S, D), A_x.dtype),
            pltpu.VMEM((seg, D), _F32),
            pltpu.VMEM((adv, D), _F32),
            pltpu.VMEM((2, M, D), _BF16),
            chunk(H * Dh, D), chunk(D, F), chunk(D, F), chunk(F, D),
            pltpu.SemaphoreType.DMA((3, n_pair)),
            pltpu.SemaphoreType.DMA((4, _SIDE_SLOTS)),
            pltpu.SemaphoreType.DMA((3,)),
            pltpu.SemaphoreType.DMA(()),
        ],
        compiler_params=pltpu.CompilerParams(vmem_limit_bytes=124 * 2**20, disable_bounds_checks=True),
    )(A_x.reshape(S, D), A_mem0.reshape(M, D), t(A_Wq), t(A_Wk), t(A_Wv), A_Wo.reshape(H * Dh, D),
      B_w_gate, B_w_up, B_w_down)
    return out.reshape(B, S, D)
```

```python
import functools
import math

import jax
import jax.numpy as jnp
import jax.experimental.pallas as pl
import jax.experimental.pallas.tpu as pltpu

_F32 = jnp.float32
_BF16 = jnp.bfloat16
_U32 = jnp.uint32
_NN = (((1,), (0,)), ((), ()))
_NT = (((1,), (1,)), ((), ()))
_LANES = 128
_SIDE_SLOTS = 3


def _mm(a, b, dims=_NN):
    return jax.lax.dot_general(a, b, dims, preferred_element_type=_F32)


def _layernorm(x):
    m = jnp.mean(x, axis=-1, keepdims=True)
    d = x - m
    v = jnp.mean(d * d, axis=-1, keepdims=True)
    return d / jnp.sqrt(v + 1e-5)


def _aligned(i, n):
    return i if isinstance(i, int) else pl.multiple_of(i, n)


def _pack(w):
    return pltpu.bitcast(w, _U32)


def _unpack(w):
    return pltpu.bitcast(w, _BF16)


def _kernel(x_hbm, mem0_hbm, wq_hbm, wk_hbm, wv_hbm, wo_hbm, wg_hbm, wu_hbm, wd_hbm, out_hbm,
            xbuf, xn0, stage, wqkv, wo, wg, wu, wd, ring0, ring1, obuf, hres, xn1, mem0,
            so, sg, su, sd, sem_w, sem_s, sem_m, sem_o, *, H, Dh, seg):
    S, D = xbuf.shape
    M = mem0_hbm.shape[0]
    F = wu_hbm.shape[1]
    n_seg = S // seg
    n_pair = H // 2
    PW = 2 * Dh
    L = M + seg
    scale = Dh ** -0.5
    adv = seg - M
    ahead = M * n_seg
    rings = (ring0, ring1)
    R = ring0.shape[1]
    off = R - ahead

    def pair_copies(p):
        rows = pl.ds(_aligned(p * PW, PW), PW)
        return [pltpu.make_async_copy(src.at[rows], stage.at[p, pl.ds(i * PW, PW)], sem_w.at[i, p])
                for i, src in enumerate((wk_hbm, wq_hbm, wv_hbm))]

    n_side = n_pair // 2 - 2
    side = ((wo_hbm, so, wo), (wg_hbm, sg, wg), (wu_hbm, su, wu), (wd_hbm, sd, wd))

    def side_start(j, src, st):
        n = st.shape[1]
        return jnp.minimum(j * n, src.shape[0] - n)

    def side_copies(j):
        slot = j % _SIDE_SLOTS
        return [pltpu.make_async_copy(src.at[pl.ds(_aligned(side_start(j, src, st), 16), st.shape[1])],
                                      st.at[slot], sem_s.at[i, slot])
                for i, (src, st, _) in enumerate(side)]

    def side_pack(j, i):
        src, st, dst = side[i]
        w = st[jnp.where(j < 0, _SIDE_SLOTS - 1, jnp.maximum(j, 0) % _SIDE_SLOTS)]
        rows = pl.ds(_aligned(side_start(jnp.maximum(j, 0), src, st) // 2, 8), st.shape[1] // 2)
        dst[rows, :] = _pack(_unpack(_pack(w.T)).T)

    def lead_pair(g, r):
        pack = ((0,), (1, 2, 3))[r]
        p = 2 * g + r
        for i in range(3):
            cols = slice(i * PW, (i + 1) * PW)
            w = stage[p, cols, :]
            rings[r][g, off:, cols] = _mm(xn0[...], w, _NT)
            wqkv[p, :, cols] = _pack(w.T)
            if i < len(pack):
                side_pack(g - 2, pack[i])

    x_head = pltpu.make_async_copy(x_hbm.at[:ahead], xbuf.at[:ahead], sem_m.at[0])
    x_tail = pltpu.make_async_copy(x_hbm.at[ahead:], xbuf.at[ahead:], sem_m.at[1])
    mem_copy = pltpu.make_async_copy(mem0_hbm, mem0.at[0], sem_m.at[2])
    x_head.start()
    mem_copy.start()
    for c in pair_copies(0):
        c.start()
    for _, st, _ in side:
        st[_SIDE_SLOTS - 1] = jnp.zeros(st.shape[1:], st.dtype)
    x_head.wait()
    xn0[...] = _layernorm(xbuf[:ahead, :].astype(_F32)).astype(_BF16)
    for c in pair_copies(1):
        c.start()

    def lead_body(p, _):
        g = p // 2
        for c in pair_copies(p):
            c.wait()

        @pl.when(p + 2 < n_pair)
        def _():
            for c in pair_copies(p + 2):
                c.start()

        @pl.when(p % 2 == 0)
        def _():
            @pl.when(g >= 2)
            def _():
                for c in side_copies(g - 2):
                    c.wait()
            lead_pair(g, 0)

        @pl.when(p % 2 == 1)
        def _():
            @pl.when(g < n_side)
            def _():
                for c in side_copies(g):
                    c.start()

            @pl.when(g == n_side)
            def _():
                x_tail.start()
            lead_pair(g, 1)
        return 0

    jax.lax.fori_loop(0, n_pair, lead_body, 0)
    x_tail.wait()
    mem_copy.wait()

    def block_diag(t):
        is_a = jax.lax.broadcasted_iota(jnp.int32, t.shape, 1) < Dh
        pad = jnp.zeros((_LANES - 2 * L, PW), _F32)
        return jnp.concatenate([jnp.where(is_a, t, 0.0), jnp.where(is_a, 0.0, t), pad], axis=0).astype(_BF16)

    def rows_of(s):
        return pl.ds(_aligned(s * seg, seg), seg)

    def out_copy(s):
        return pltpu.make_async_copy(obuf.at[rows_of(s)], out_hbm.at[rows_of(s)], sem_o)

    def ffn_gate(hn):
        g = _mm(hn, _unpack(wg[...]))
        return g * jax.nn.sigmoid(g)

    def ffn_up(hn, cols=slice(None)):
        return _mm(hn, _unpack(wu[:, cols]))

    def ffn_down(s, a):
        y = hres[...] + _mm(a.astype(_BF16), _unpack(wd[...]))
        obuf[rows_of(s), :] = y.astype(obuf.dtype)

    def ln_new(s):
        return _layernorm(xbuf[pl.ds(_aligned(ahead + s * adv, M), adv), :].astype(_F32))

    def step(s, mem):
        h = jnp.concatenate([mem, xn1[...]], axis=0).astype(_BF16)
        xn1[...] = ln_new(jnp.minimum(s + 1, n_seg - 1))
        put = pl.ds(pl.multiple_of(jax.lax.rem(s * adv, R), M), adv)
        get = pl.ds(pl.multiple_of(jax.lax.rem(s * seg + off, R), seg), seg)
        hn = _layernorm(hres[...]).astype(_BF16)

        row = jax.lax.broadcasted_iota(jnp.int32, (L, _LANES), 0)
        col = jax.lax.broadcasted_iota(jnp.int32, (L, _LANES), 1)
        head_a = col < L
        head_b = (col >= L) & (col < 2 * L)
        key = jnp.where(head_a, col, col - L)
        allowed = ((row < M) | (row >= key)) & (col < 2 * L)
        fill = jnp.where(col < 2 * L, -1e9, -jnp.inf)

        def proj(p):
            kqv = _mm(h, _unpack(wqkv[p]))
            ring = rings[p % 2]
            ring[p // 2, put, :] = kqv[M:]
            kqv = jnp.concatenate([kqv[:M], ring[p // 2, get, :]], axis=0)
            return kqv[:, :PW], kqv[:, PW:2 * PW], kqv[:, 2 * PW:]

        def probs(q, k):
            sc = _mm(q, block_diag(k), _NT) * scale
            sc = jnp.where(allowed, sc, fill)
            m_a = jnp.max(jnp.where(head_a, sc, -jnp.inf), axis=-1, keepdims=True)
            m_b = jnp.max(jnp.where(head_b, sc, -jnp.inf), axis=-1, keepdims=True)
            e = jnp.exp(sc - jnp.where(head_a, m_a, m_b))
            l_a = jnp.sum(jnp.where(head_a, e, 0.0), axis=-1, keepdims=True)
            l_b = jnp.sum(jnp.where(head_b, e, 0.0), axis=-1, keepdims=True)
            return e / jnp.where(head_a, l_a, l_b)

        kqv, v, prob, o = {}, {}, {}, {}
        acc = None
        half = F // 2
        for i in range(n_pair + 3):
            if i < n_pair:
                kqv[i] = proj(i)
            elif i == n_pair:
                g = ffn_gate(hn)
            elif i == n_pair + 1:
                a0 = g[:, :half] * ffn_up(hn, slice(0, half))
            else:
                a1 = g[:, half:] * ffn_up(hn, slice(half, F))
            if i >= 3:
                c = _mm(o.pop(i - 3), _unpack(wo[(i - 3) * Dh:(i - 2) * Dh, :]))
                acc = c if acc is None else acc + c
            if 1 <= i <= n_pair:
                k, q, v[i - 1] = kqv.pop(i - 1)
                prob[i - 1] = probs(q, k)
            if 2 <= i <= n_pair + 1:
                o[i - 2] = _mm(prob.pop(i - 2), block_diag(v.pop(i - 2)))
        ffn_down(jnp.maximum(s - 1, 0), jnp.concatenate([a0, a1], axis=1))
        hres[...] = xbuf[rows_of(s), :].astype(_F32) + acc[M:]

        @pl.when(s > 0)
        def _():
            out_copy(s - 1).start()
        return acc[:M]

    hres[...] = jnp.zeros(hres.shape, _F32)
    xn1[...] = ln_new(0)
    jax.lax.fori_loop(0, n_seg, step, mem0[0].astype(_F32), unroll=4)
    hn = _layernorm(hres[...]).astype(_BF16)
    ffn_down(n_seg - 1, ffn_gate(hn) * ffn_up(hn))
    out_copy(n_seg - 1).start()
    pltpu.make_async_copy(obuf, out_hbm, sem_o).wait()


@functools.partial(jax.jit, static_argnames=("A_seg_len",))
def pallas_sequential_preLN__memory_aug_recurrent_mem_tr__swiglu_ffn__prompt_kernel(
    A_x: jax.Array,
    A_mem0: jax.Array,
    A_Wq: jax.Array,
    A_Wk: jax.Array,
    A_Wv: jax.Array,
    A_Wo: jax.Array,
    A_seg_len: int,
    B_x: jax.Array,
    B_w_gate: jax.Array,
    B_w_up: jax.Array,
    B_w_down: jax.Array,
):
    del B_x
    B, S, D = A_x.shape
    _, H, Dh = A_Wq.shape
    M = A_mem0.shape[1]
    F = B_w_gate.shape[1]
    seg = int(A_seg_len)
    n_pair = H // 2
    adv, ahead = seg - M, M * (S // seg)
    period = math.lcm(adv, seg)
    ring_rows = period * pl.cdiv(ahead + adv, period)
    assert B == 1 and S % seg == 0 and H % 4 == 0 and n_pair > 4
    assert M % 8 == 0 and seg % 16 == 0 and ahead % seg == 0 and 2 * (M + seg) <= _LANES

    def t(w):
        return jnp.transpose(w, (1, 2, 0)).reshape(H * Dh, D)

    def chunk(rows, cols):
        return pltpu.VMEM((_SIDE_SLOTS, 16 * pl.cdiv(rows, 16 * (n_pair // 2 - 2)), cols), _BF16)

    hbm = pl.BlockSpec(memory_space=pl.ANY)
    out = pl.pallas_call(
        functools.partial(_kernel, H=H, Dh=Dh, seg=seg),
        out_shape=jax.ShapeDtypeStruct((S, D), A_x.dtype),
        in_specs=[hbm] * 9,
        out_specs=hbm,
        scratch_shapes=[
            pltpu.VMEM((S, D), _BF16),
            pltpu.VMEM((ahead, D), _BF16),
            pltpu.VMEM((n_pair, 6 * Dh, D), _BF16),
            pltpu.VMEM((n_pair, D // 2, 6 * Dh), _U32),
            pltpu.VMEM((H * Dh // 2, D), _U32),
            pltpu.VMEM((D // 2, F), _U32),
            pltpu.VMEM((D // 2, F), _U32),
            pltpu.VMEM((F // 2, D), _U32),
            pltpu.VMEM((n_pair // 2, ring_rows, 6 * Dh), _F32),
            pltpu.VMEM((n_pair // 2, ring_rows, 6 * Dh), _F32),
            pltpu.VMEM((S, D), A_x.dtype),
            pltpu.VMEM((seg, D), _F32),
            pltpu.VMEM((adv, D), _F32),
            pltpu.VMEM((2, M, D), _BF16),
            chunk(H * Dh, D), chunk(D, F), chunk(D, F), chunk(F, D),
            pltpu.SemaphoreType.DMA((3, n_pair)),
            pltpu.SemaphoreType.DMA((4, _SIDE_SLOTS)),
            pltpu.SemaphoreType.DMA((3,)),
            pltpu.SemaphoreType.DMA(()),
        ],
        compiler_params=pltpu.CompilerParams(vmem_limit_bytes=124 * 2**20, disable_bounds_checks=True),
    )(A_x.reshape(S, D), A_mem0.reshape(M, D), t(A_Wq), t(A_Wk), t(A_Wv), A_Wo.reshape(H * Dh, D),
      B_w_gate, B_w_up, B_w_down)
    return out.reshape(B, S, D)
```
